```python
import os as _os
_os.environ.setdefault('JAX_PLATFORMS', 'cpu')
import jax
import jax.numpy as jnp

def _softmax(x, axis=-1):
    return jax.nn.softmax(x, axis=axis)

def _gelu(x):
    return jax.nn.gelu(x, approximate=True)

def _silu(x):
    return jax.nn.silu(x)

def _sigmoid(x):
    return jax.nn.sigmoid(x)

def _layernorm(x, axis=-1, eps=1e-05):
    m = jnp.mean(x, axis=axis, keepdims=True)
    v = jnp.var(x, axis=axis, keepdims=True)
    return (x - m) / jnp.sqrt(v + eps)

def _scatter_add(tgt, idx, src, axis=0):
    return tgt.at[idx].add(src)

def _segment_sum(src, seg, n):
    return jax.ops.segment_sum(src, seg, n)

class _Rng:

    def __init__(self, key):
        self._k = key

    def _next(self):
        self._k, sub = jax.random.split(self._k)
        return sub

    def normal(self, shape):
        return jax.random.normal(self._next(), shape, dtype=jnp.bfloat16)

    def randint(self, lo, hi, shape):
        return jax.random.randint(self._next(), shape, lo, hi, dtype=jnp.int32)

    def uniform(self, shape, lo=0.0, hi=1.0):
        return jax.random.uniform(self._next(), shape, jnp.bfloat16, lo, hi)

    def permutation(self, n):
        return jax.random.permutation(self._next(), n)
kernel_name = 'sequential_preLN__memory_aug_recurrent_mem_tr__swiglu_ffn__prompt'

def setup_inputs():
    _rng = _Rng(jax.random.key(int.from_bytes(__import__("os").urandom(4), "little")))
    _w = lambda a: (lambda t: t.astype(jnp.bfloat16) if jnp.issubdtype(t.dtype, jnp.floating) else t)(jnp.asarray(a))

    def _A_setup():
        B, S, Dm = (1, 2048, 640)
        H, Dh = (32, 192)
        M, seg = (8, 32)
        seg = min(seg, S)
        S = S // seg * seg
        return {'x': _w((lambda *s: _rng.normal(s) * 0.05)(B, S, Dm)), 'mem0': _w((lambda *s: _rng.normal(s) * 0.1)(B, M, Dm)), 'Wq': _w((lambda *s: _rng.normal(s) * 1.6)(Dm, H, Dh) * Dm ** (-0.5)), 'Wk': _w((lambda *s: _rng.normal(s) * 1.6)(Dm, H, Dh) * Dm ** (-0.5)), 'Wv': _w((lambda *s: _rng.normal(s) * 0.1)(Dm, H, Dh) * Dm ** (-0.5)), 'Wo': _w((lambda *s: _rng.normal(s) * 0.1)(H, Dh, Dm) * (H * Dh) ** (-0.5)), 'seg_len': seg}
    _A_in = _A_setup()

    def _B_setup():
        B, S, D, F = (1, 2048, 640, 1536)
        return {'x': _w((lambda *s: _rng.normal(s) * 0.05)(B, S, D)), 'w_gate': _w((lambda *s: _rng.normal(s) * 0.05)(D, F)), 'w_up': _w((lambda *s: _rng.normal(s) * 0.05)(D, F)), 'w_down': _w((lambda *s: _rng.normal(s) * 0.05)(F, D))}
    _B_in = _B_setup()
    return {'A_x': _A_in['x'], 'A_mem0': _A_in['mem0'], 'A_Wq': _A_in['Wq'], 'A_Wk': _A_in['Wk'], 'A_Wv': _A_in['Wv'], 'A_Wo': _A_in['Wo'], 'A_seg_len': _A_in['seg_len'], 'B_x': _B_in['x'], 'B_w_gate': _B_in['w_gate'], 'B_w_up': _B_in['w_up'], 'B_w_down': _B_in['w_down']}

def reference(A_x, A_mem0, A_Wq, A_Wk, A_Wv, A_Wo, A_seg_len, B_x, B_w_gate, B_w_up, B_w_down):

    def _A_ref(x, mem0, Wq, Wk, Wv, Wo, seg_len):
        B, S, Dm = x.shape
        H, Dh = (Wq.shape[1], Wq.shape[2])
        M = mem0.shape[1]
        scale = Dh ** (-0.5)
        n_seg = S // seg_len
        L = M + seg_len
        idx = jnp.arange(L)
        mask = (idx[:, None] < M) | (idx[:, None] >= idx[None, :])
        mem = mem0
        outs = []
        for s in range(n_seg):
            xs = x[:, s * seg_len:(s + 1) * seg_len, :].copy()
            h = jnp.concatenate([mem, xs], axis=1)
            q = jnp.einsum('btd,dhe->bhte', h, Wq)
            k = jnp.einsum('btd,dhe->bhte', h, Wk)
            v = jnp.einsum('btd,dhe->bhte', h, Wv)
            scores = jnp.einsum('bhqe,bhke->bhqk', q, k) * scale
            scores = jnp.where(mask[None, None], scores, -1000000000.0)
            p = _softmax(scores, axis=-1)
            o = jnp.einsum('bhqk,bhke->bhqe', p, v)
            o = jnp.einsum('bhte,hed->btd', o, Wo)
            mem = o[:, :M, :].copy()
            outs.append(o[:, M:, :])
        return jnp.concatenate(outs, axis=1)

    def _B_ref(x, w_gate, w_up, w_down):
        g = _silu(x @ w_gate)
        u = x @ w_up
        return g * u @ w_down
    x = A_x
    h = x + _A_ref(_layernorm(x, axis=-1), A_mem0, A_Wq, A_Wk, A_Wv, A_Wo, A_seg_len)
    h2 = h + _B_ref(_layernorm(h, axis=-1), B_w_gate, B_w_up, B_w_down)
    return h2
```

```python
import functools
import numpy as np
import jax
import jax.numpy as jnp
from jax.experimental import pallas as pl
from jax.experimental.pallas import tpu as pltpu

F32 = jnp.float32
BF16 = jnp.bfloat16
LOG2E = 1.4426950408889634
UNROLL = 3
AHEAD = 4


def _ln(x):
    m = jnp.mean(x, axis=-1, keepdims=True)
    d = x - m
    v = jnp.mean(d * d, axis=-1, keepdims=True)
    return d * jax.lax.rsqrt(v + 1e-5)


def _mm(a, b):
    return jax.lax.dot_general(a, b, (((1,), (0,)), ((), ())), preferred_element_type=F32)


def _mm_nt(a, b):
    return jax.lax.dot_general(a, b, (((1,), (1,)), ((), ())), preferred_element_type=F32)


def _kernel(x_hbm, mem0_ref, wq_hbm, wk_hbm, wv_hbm, wo_hbm, wg_hbm, wu_hbm, wd_hbm, out_hbm,
            stage, wqkv, wo, wg, wu, wd, xv, xg, xgn, pre, outv, h_scr, hres,
            sem_w, sem_wo, sem_m, sem_x, sem_o,
            *, M, SEG, NSEG, DH, NP, TP):
    L = M + SEG
    LK = L - TP
    PW = 2 * DH
    D = xv.shape[2]
    F = wg.shape[1]
    FH = F // 2
    c = (DH ** -0.5) * LOG2E
    U = UNROLL
    NIT = (NSEG - 1) // U

    def w_copy(p, j):
        src = (wk_hbm, wv_hbm, wq_hbm)[j]
        return pltpu.make_async_copy(src.at[pl.ds(pl.multiple_of(p * PW, PW), PW), :], stage.at[p * 3 + j],
                                     sem_w.at[p * 3 + j])

    def wo_copy(p):
        r = pl.ds(pl.multiple_of(p * PW, PW), PW)
        return pltpu.make_async_copy(wo_hbm.at[r, :], wo.at[r, :], sem_wo.at[p])

    def x_copy(s0, n, slot):
        return pltpu.make_async_copy(x_hbm.at[pl.ds(s0, n)], xv.at[pl.ds(s0, n)], sem_x.at[slot])

    xg_copy = pltpu.make_async_copy(x_hbm.at[:, pl.ds(SEG - TP, TP), :], xg, sem_m.at[0])
    ffn_copies = [pltpu.make_async_copy(wg_hbm, wg, sem_m.at[1]),
                  pltpu.make_async_copy(wu_hbm, wu, sem_m.at[2]),
                  pltpu.make_async_copy(wd_hbm, wd, sem_m.at[3])]
    x0_copy = x_copy(0, 2 + U, 1)

    xg_copy.start()
    w_copy(0, 0).start()
    w_copy(0, 1).start()
    xg_copy.wait()
    w_copy(0, 2).start()
    for j in range(3):
        w_copy(1, j).start()
    xgn[...] = _ln(xg[...].astype(F32).reshape(NSEG * TP, D)).astype(BF16)

    def wait_pair(p):
        for j in range(3):
            w_copy(p, j).wait()

    def transpose_piece(p, j, r):
        t = stage[p * 3 + j, r * 128:(r + 1) * 128, :].T
        wqkv[p, :, j * PW + r * 128:j * PW + (r + 1) * 128] = t
        return t

    def fused(tr, mm):
        pieces = [(j, r) for j in range(3) for r in range(3)]
        for n in range(6):
            deps = []
            if tr is not None:
                k0, k1 = ((0, 0), (0, 2), (2, 4), (4, 6), (6, 8), (8, 9))[n]
                for (j, r) in pieces[k0:k1]:
                    deps.append(transpose_piece(tr, j, r))
            if mm is not None:
                w = wqkv[mm, :, n * 128:(n + 1) * 128]
                for t in deps:
                    w = jnp.where(mm < 0, t, w)
                pre[mm, :, n * 128:(n + 1) * 128] = _mm(xgn[...], w)

    wait_pair(0)
    for p in range(2, AHEAD):
        for j in range(3):
            w_copy(p, j).start()
    x0_copy.start()
    fused(0, None)

    def pre_body(p, carry):
        @pl.when(p + AHEAD < NP)
        def _():
            for j in range(3):
                w_copy(p + AHEAD, j).start()
            wo_copy(p).start()

        @pl.when(p + AHEAD == NP)
        def _():
            for q in range(NP - AHEAD, NP):
                wo_copy(q).start()
        wait_pair(p + 1)
        fused(p + 1, p)
        return carry
    jax.lax.fori_loop(0, NP - 1, pre_body, 0)
    for cp in ffn_copies:
        cp.start()
    x0_copy.wait()
    h_scr[0:M, :] = mem0_ref[...].astype(F32)
    h_scr[M:L, :] = _ln(xv[0].astype(F32))
    fused(None, NP - 1)
    for p in range(NP):
        wo_copy(p).wait()

    def out_copy(s0, n):
        return pltpu.make_async_copy(outv.at[pl.ds(s0, n)], out_hbm.at[pl.ds(s0, n)], sem_o.at[0])

    def bdiag(t):
        lo = jax.lax.broadcasted_iota(jnp.int32, (L, PW), 1) < DH
        return jnp.concatenate([jnp.where(lo, t, 0.0), jnp.where(lo, 0.0, t)], axis=0).astype(BF16)

    def softmax(s):
        s = s * c
        row = jax.lax.broadcasted_iota(jnp.int32, (L, 2 * L), 0)
        col = jax.lax.broadcasted_iota(jnp.int32, (L, 2 * L), 1)
        first = col < L
        key = jnp.where(first, col, col - L)
        s = jnp.where((row < M) | (row >= key), s, -1e9 * LOG2E)
        m1 = jnp.max(jnp.where(first, s, -jnp.inf), axis=-1, keepdims=True)
        m2 = jnp.max(jnp.where(first, -jnp.inf, s), axis=-1, keepdims=True)
        e = jnp.exp2(s - jnp.where(first, m1, m2))
        l1 = jnp.sum(jnp.where(first, e, 0.0), axis=-1, keepdims=True)
        l2 = jnp.sum(jnp.where(first, 0.0, e), axis=-1, keepdims=True)
        return e / jnp.where(first, l1, l2)

    def swiglu(g, u):
        return g * jax.nn.sigmoid(g) * u

    def step(s, with_ffn):
        h = h_scr[...]
        hk = h[0:LK]
        rows = pl.ds(pl.multiple_of(s * TP, TP), TP)

        def proj(p):
            k = _mm(hk, wqkv[p, :, 0:PW])
            q = _mm(h, wqkv[p, :, 2 * PW:3 * PW])
            v = _mm(hk, wqkv[p, :, PW:2 * PW])
            k = jnp.concatenate([k, pre[p, rows, 0:PW]], axis=0)
            v = jnp.concatenate([v, pre[p, rows, PW:2 * PW]], axis=0)
            return q, k, v

        def wo_mm(o, p):
            return _mm(o, wo[p * PW:(p + 1) * PW, :])

        q, k, v = proj(0)
        if with_ffn:
            hr = hres[...]
            hn = _ln(hr)
            g1 = _mm(hn, wg[:, 0:FH])
        acc = None
        o_prev = None
        for p in range(NP):
            sc = _mm_nt(q, bdiag(k))
            nxt = None
            if p + 1 < NP:
                nxt = proj(p + 1)
            elif with_ffn:
                act2 = swiglu(_mm(hn, wg[:, FH:F]), _mm(hn, wu[:, FH:F]))
            if p == 0:
                if with_ffn:
                    act1 = swiglu(g1, _mm(hn, wu[:, 0:FH]))
            else:
                t = wo_mm(o_prev, p - 1)
                acc = t if acc is None else acc + t
            o_prev = _mm(softmax(sc), bdiag(v))
            if nxt is not None:
                q, k, v = nxt
        if with_ffn:
            y = hr + _mm(act1, wd[0:FH, :])
        acc = acc + wo_mm(o_prev, NP - 1)
        sn = jnp.minimum(s + 1, NSEG - 1)
        h_scr[0:M, :] = acc[0:M, :]
        h_scr[M:L, :] = _ln(xv[sn].astype(F32))
        hres[...] = xv[s].astype(F32) + acc[M:L, :]
        if with_ffn:
            outv[s - 1] = (y + _mm(act2, wd[FH:F, :])).astype(BF16)

    step(0, False)
    for cp in ffn_copies:
        cp.wait()

    x1_copy = x_copy(2 + U, NSEG - 2 - U, 0)
    x1_copy.start()

    def body(i, carry):
        @pl.when(i == 1)
        def _():
            x1_copy.wait()

        @pl.when(i > 0)
        def _():
            out_copy((i - 1) * U, U).start()
        for u in range(U):
            step(1 + i * U + u, True)
        return carry
    jax.lax.fori_loop(0, NIT, body, 0)

    out_copy((NIT - 1) * U, U).start()
    hr = hres[...]
    hn = _ln(hr)
    act1 = swiglu(_mm(hn, wg[:, 0:FH]), _mm(hn, wu[:, 0:FH]))
    act2 = swiglu(_mm(hn, wg[:, FH:F]), _mm(hn, wu[:, FH:F]))
    outv[NSEG - 1] = (hr + _mm(act1, wd[0:FH, :]) + _mm(act2, wd[FH:F, :])).astype(BF16)
    out_copy(NSEG - 1, 1).start()
    pltpu.make_async_copy(outv, out_hbm, sem_o.at[0]).wait()


@functools.partial(jax.jit, static_argnames=("A_seg_len",))
def pallas_sequential_preLN__memory_aug_recurrent_mem_tr__swiglu_ffn__prompt_kernel(A_x, A_mem0, A_Wq, A_Wk, A_Wv, A_Wo, A_seg_len, B_x, B_w_gate, B_w_up, B_w_down):
    B, S, D = A_x.shape
    H, DH = A_Wq.shape[1], A_Wq.shape[2]
    M = A_mem0.shape[1]
    SEG = int(A_seg_len)
    NSEG = S // SEG
    F = B_w_gate.shape[1]
    NP = H // 2
    PW = 2 * DH
    TP = 8
    tw = lambda w: jnp.transpose(w, (1, 2, 0)).reshape(H * DH, D)
    any_spec = pl.BlockSpec(memory_space=pl.ANY)
    out = pl.pallas_call(
        functools.partial(_kernel, M=M, SEG=SEG, NSEG=NSEG, DH=DH, NP=NP, TP=TP),
        out_shape=jax.ShapeDtypeStruct((NSEG, SEG, D), A_x.dtype),
        in_specs=[any_spec, pl.BlockSpec(memory_space=pltpu.VMEM)] + [any_spec] * 7,
        out_specs=any_spec,
        scratch_shapes=[
            pltpu.VMEM((NP * 3, PW, D), BF16),
            pltpu.VMEM((NP, D, 3 * PW), BF16),
            pltpu.VMEM((H * DH, D), BF16),
            pltpu.VMEM((D, F), BF16),
            pltpu.VMEM((D, F), BF16),
            pltpu.VMEM((F, D), BF16),
            pltpu.VMEM((NSEG, SEG, D), BF16),
            pltpu.VMEM((NSEG, TP, D), BF16),
            pltpu.VMEM((NSEG * TP, D), BF16),
            pltpu.VMEM((NP, NSEG * TP, 2 * PW), F32),
            pltpu.VMEM((NSEG, SEG, D), BF16),
            pltpu.VMEM((M + SEG, D), F32),
            pltpu.VMEM((SEG, D), F32),
            pltpu.SemaphoreType.DMA((NP * 3,)),
            pltpu.SemaphoreType.DMA((NP,)),
            pltpu.SemaphoreType.DMA((4,)),
            pltpu.SemaphoreType.DMA((2,)),
            pltpu.SemaphoreType.DMA((1,)),
        ],
        compiler_params=pltpu.CompilerParams(vmem_limit_bytes=120 * 1024 * 1024),
    )(A_x.reshape(NSEG, SEG, D), A_mem0.reshape(M, D), tw(A_Wq), tw(A_Wk), tw(A_Wv), A_Wo.reshape(H * DH, D),
      B_w_gate, B_w_up, B_w_down)
    return out.reshape(B, S, D)
```

```python
import functools

import jax
import jax.numpy as jnp
from jax.experimental import pallas as pl
from jax.experimental.pallas import tpu as pltpu

F32 = jnp.float32
BF16 = jnp.bfloat16
U32 = jnp.uint32
LOG2E = 1.4426950408889634
LANES = 128
UNROLL = 3
AHEAD = 3
TP = 8


def _ln(x):
    m = jnp.mean(x, axis=-1, keepdims=True)
    d = x - m
    v = jnp.mean(d * d, axis=-1, keepdims=True)
    return d * jax.lax.rsqrt(v + 1e-5)


def _mm(a, b):
    return jax.lax.dot_general(a, b, (((1,), (0,)), ((), ())), preferred_element_type=F32)


def _mm_packed(a, b):
    return _mm(a, pltpu.bitcast(b, BF16))


def _mm_nt(a, b):
    return jax.lax.dot_general(a, b, (((1,), (1,)), ((), ())), preferred_element_type=F32)


def _swiglu(g, u):
    return g * jax.nn.sigmoid(g) * u


def _kernel(x_hbm, mem0_ref, wq_hbm, wk_hbm, wv_hbm, wo_hbm, wg_hbm, wu_hbm, wd_hbm, out_hbm,
            stage, wkvq, wo, wg, wu, wd, xv, xg, xgn, pre, outv, h_scr, hres,
            sem_w, sem_wo, sem_m, sem_x, sem_o, *, DH):
    NSEG, SEG, D = x_hbm.shape
    M = mem0_ref.shape[0]
    NP = wkvq.shape[0]
    PW = 2 * DH
    PT = PW // LANES
    L = M + SEG
    LK = L - TP
    F = wg.shape[1]
    FH = F // 2
    NIT = (NSEG - 1) // UNROLL
    K, V, Q = range(3)

    def w_copy(p, j):
        src = (wk_hbm, wv_hbm, wq_hbm)[j]
        return pltpu.make_async_copy(src.at[pl.ds(pl.multiple_of(p * PW, PW), PW), :],
                                     stage.at[p * 3 + j], sem_w.at[p * 3 + j])

    def wo_copy(p):
        r = pl.ds(pl.multiple_of(p * PW, PW), PW)
        return pltpu.make_async_copy(wo_hbm.at[r, :], wo.at[r, :], sem_wo.at[p])

    def x_start(i):
        return jnp.minimum(1 + i * UNROLL, NSEG - UNROLL - 1)

    def x_copy(i):
        slot = i % 2
        return pltpu.make_async_copy(x_hbm.at[pl.ds(x_start(i), UNROLL + 1)], xv.at[slot], sem_x.at[slot])

    def out_copy(s):
        return pltpu.make_async_copy(outv.at[pl.ds(s, 1)], out_hbm.at[pl.ds(s, 1)], sem_o.at[0])

    def group(p):
        return [w_copy(p + 1, K), w_copy(p, V)]

    xg_copy = pltpu.make_async_copy(x_hbm.at[:, pl.ds(SEG - TP, TP), :], xg, sem_m.at[0])
    x0_copy = pltpu.make_async_copy(x_hbm.at[pl.ds(0, 2)], xv.at[1, pl.ds(0, 2)], sem_x.at[1])
    ffn_copies = [pltpu.make_async_copy(wg_hbm, wg, sem_m.at[1]),
                  pltpu.make_async_copy(wu_hbm, wu, sem_m.at[2]),
                  pltpu.make_async_copy(wd_hbm, wd, sem_m.at[3])]

    def transpose_piece(src, p, j, r):
        t = pltpu.bitcast(stage[src, r * LANES:(r + 1) * LANES, :].T, U32)
        wkvq[p, :, j * PW + r * LANES:j * PW + (r + 1) * LANES] = t
        return t

    def pre_piece(p, n, pieces=(), never=None, chunks=4):
        cols = slice(n * LANES, (n + 1) * LANES)
        deps = [transpose_piece(*piece) for piece in pieces]
        w = wkvq[p, :, cols]
        for t in deps:
            w = jnp.where(never, t, w)
        w = pltpu.bitcast(w, BF16)
        rc = NSEG * TP // chunks
        for r in range(chunks):
            pre[p, r * rc:(r + 1) * rc, cols] = _mm(xgn[r * rc:(r + 1) * rc, :], w)

    xg_copy.start()
    w_copy(0, K).start()
    xg_copy.wait()
    for cp in group(0):
        cp.start()
    w_copy(0, K).wait()
    xgn[...] = _ln(xg[...].astype(F32).reshape(NSEG * TP, D)).astype(BF16)
    for r in range(PT):
        transpose_piece(K, 0, K, r)
    for p in range(1, AHEAD):
        for cp in group(p):
            cp.start()
        w_copy(p - 1, Q).start()
    x0_copy.start()
    x_copy(0).start()

    def pre_body(p, carry):
        @pl.when(p + AHEAD < NP - 1)
        def _():
            for cp in group(p + AHEAD):
                cp.start()
            w_copy(p + AHEAD - 1, Q).start()
            wo_copy(p).start()

        @pl.when(p + AHEAD == NP - 1)
        def _():
            w_copy(NP - 1, V).start()
            w_copy(NP - 2, Q).start()
            w_copy(NP - 1, Q).start()
            for pp in range(NP - 1 - AHEAD, NP):
                wo_copy(pp).start()

        @pl.when(p > 0)
        def _():
            w_copy(p - 1, Q).wait()

        for cp in group(p):
            cp.wait()
        qp = jnp.maximum(p - 1, 0)
        qsrc = jnp.where(p > 0, qp * 3 + Q, K)
        kk = [((p + 1) * 3 + K, p + 1, K, r) for r in range(PT)]
        qq = [(qsrc, qp, Q, r) for r in range(PT)]
        deps = ([], kk[0:1], kk[1:2], kk[2:3] + qq[0:1], qq[1:2], qq[2:3])
        for r in range(PT):
            transpose_piece(p * 3 + V, p, V, r)
        for n in range(2 * PT):
            pre_piece(p, n, deps[n], p < 0, 1)
        return carry

    jax.lax.fori_loop(0, NP - 1, pre_body, 0)

    for cp in ffn_copies:
        cp.start()
    x0_copy.wait()
    w_copy(NP - 1, V).wait()
    w_copy(NP - 2, Q).wait()
    w_copy(NP - 1, Q).wait()
    for p in range(NP):
        wo_copy(p).wait()
    h_scr[0:M, :] = mem0_ref[...].astype(F32)
    h_scr[M:L, :] = _ln(xv[1, 0].astype(F32))
    for r in range(PT):
        transpose_piece((NP - 1) * 3 + V, NP - 1, V, r)

    def block_diag(t):
        first = jax.lax.broadcasted_iota(jnp.int32, (L, PW), 1) < DH
        return jnp.concatenate([jnp.where(first, t, 0.0), jnp.where(first, 0.0, t)], axis=0).astype(BF16)

    def softmax(s):
        s = s * (DH ** -0.5 * LOG2E)
        row = jax.lax.broadcasted_iota(jnp.int32, (L, 2 * L), 0)
        col = jax.lax.broadcasted_iota(jnp.int32, (L, 2 * L), 1)
        first = col < L
        key = jnp.where(first, col, col - L)
        s = jnp.where((row < M) | (row >= key), s, -1e9 * LOG2E)
        m1 = jnp.max(jnp.where(first, s, -jnp.inf), axis=-1, keepdims=True)
        m2 = jnp.max(jnp.where(first, -jnp.inf, s), axis=-1, keepdims=True)
        e = jnp.exp2(s - jnp.where(first, m1, m2))
        l1 = jnp.sum(jnp.where(first, e, 0.0), axis=-1, keepdims=True)
        l2 = jnp.sum(jnp.where(first, 0.0, e), axis=-1, keepdims=True)
        return e / jnp.where(first, l1, l2)

    def step(s, x_cur, x_next, first_step):
        h = h_scr[...]
        hk = h[0:LK]
        rows = pl.ds(pl.multiple_of(s * TP, TP), TP)
        last = NP - 1

        def proj(p):
            direct = first_step and p == last
            k = _mm_packed(h if direct else hk, wkvq[p, :, K * PW:(K + 1) * PW])
            q = _mm_packed(h, wkvq[p, :, Q * PW:(Q + 1) * PW])
            v = _mm_packed(h if direct else hk, wkvq[p, :, V * PW:(V + 1) * PW])
            if not direct:
                k = jnp.concatenate([k, pre[p, rows, K * PW:(K + 1) * PW]], axis=0)
                v = jnp.concatenate([v, pre[p, rows, V * PW:(V + 1) * PW]], axis=0)
            return q, k, v

        def out_proj(o, p):
            return _mm(o, wo[p * PW:(p + 1) * PW, :])

        def wq_pieces(p):
            return [(p * 3 + Q, p, Q, r) for r in range(PT)]

        if first_step:
            never = pl.program_id(0) < 0
            pre_piece(last, 0)
        q, k, v = proj(0)
        if first_step:
            pre_piece(last, 1, wq_pieces(last - 1), never)
        else:
            hr = hres[...]
            hn = _ln(hr)
            g1 = _mm(hn, wg[:, 0:FH])
        for p in range(NP):
            scores = _mm_nt(q, block_diag(k))
            if p < last:
                nxt = proj(p + 1)
            elif first_step:
                pre_piece(last, 3)
            else:
                act2 = _swiglu(_mm(hn, wg[:, FH:F]), _mm(hn, wu[:, FH:F]))
            if p > 0:
                t = out_proj(o, p - 1)
                acc = t if p == 1 else acc + t
            elif first_step:
                pre_piece(last, 2, wq_pieces(last), never)
            else:
                act1 = _swiglu(g1, _mm(hn, wu[:, 0:FH]))
            o = _mm(softmax(scores), block_diag(v))
            if p < last:
                q, k, v = nxt
        if first_step:
            pre_piece(last, 4)
        else:
            y = hr + _mm(act1, wd[0:FH, :])
        acc = acc + out_proj(o, last)
        h_scr[0:M, :] = acc[0:M, :]
        h_scr[M:L, :] = _ln(x_next().astype(F32))
        hres[...] = x_cur().astype(F32) + acc[M:L, :]
        if first_step:
            pre_piece(last, 5)
        else:
            outv[s - 1] = (y + _mm(act2, wd[FH:F, :])).astype(BF16)
            out_copy(s - 1).start()

    step(0, lambda: xv[1, 0], lambda: xv[1, 1], True)
    for cp in ffn_copies:
        cp.wait()

    def body(i, carry):
        x_copy(i).wait()
        x_copy(i + 1).start()
        off = 1 + i * UNROLL - x_start(i)
        slot = i % 2
        for u in range(UNROLL):
            step(1 + i * UNROLL + u, lambda: xv[slot, off + u],
                 lambda: xv[slot, jnp.minimum(off + u + 1, UNROLL)], False)
        return carry

    jax.lax.fori_loop(0, NIT, body, 0)

    x_copy(NIT).wait()
    hr = hres[...]
    hn = _ln(hr)
    act1 = _swiglu(_mm(hn, wg[:, 0:FH]), _mm(hn, wu[:, 0:FH]))
    act2 = _swiglu(_mm(hn, wg[:, FH:F]), _mm(hn, wu[:, FH:F]))
    outv[NSEG - 1] = (hr + _mm(act1, wd[0:FH, :]) + _mm(act2, wd[FH:F, :])).astype(BF16)
    out_copy(NSEG - 1).start()
    pltpu.make_async_copy(outv, out_hbm, sem_o.at[0]).wait()


@functools.partial(jax.jit, static_argnames=("A_seg_len",))
def pallas_sequential_preLN__memory_aug_recurrent_mem_tr__swiglu_ffn__prompt_kernel(
    A_x: jax.Array,
    A_mem0: jax.Array,
    A_Wq: jax.Array,
    A_Wk: jax.Array,
    A_Wv: jax.Array,
    A_Wo: jax.Array,
    A_seg_len: int,
    B_x: jax.Array,
    B_w_gate: jax.Array,
    B_w_up: jax.Array,
    B_w_down: jax.Array,
):
    B, S, D = A_x.shape
    H, DH = A_Wq.shape[1], A_Wq.shape[2]
    M = A_mem0.shape[1]
    SEG = int(A_seg_len)
    NSEG = S // SEG
    F = B_w_gate.shape[1]
    NP = H // 2
    PW = 2 * DH
    assert B == 1 and S == NSEG * SEG and H == 2 * NP and PW == 3 * LANES
    assert (NSEG - 1) % UNROLL == 0 and SEG > TP and NP > AHEAD + 1

    def heads_major(w):
        return jnp.transpose(w, (1, 2, 0)).reshape(H * DH, D)

    any_spec = pl.BlockSpec(memory_space=pl.ANY)
    out = pl.pallas_call(
        functools.partial(_kernel, DH=DH),
        grid=(1,),
        out_shape=jax.ShapeDtypeStruct((NSEG, SEG, D), A_x.dtype),
        in_specs=[any_spec, pl.BlockSpec((M, D), lambda i: (0, 0))] + [any_spec] * 7,
        out_specs=any_spec,
        scratch_shapes=[
            pltpu.VMEM((NP * 3, PW, D), BF16),
            pltpu.VMEM((NP, D // 2, 3 * PW), U32),
            pltpu.VMEM((H * DH, D), BF16),
            pltpu.VMEM((D, F), BF16),
            pltpu.VMEM((D, F), BF16),
            pltpu.VMEM((F, D), BF16),
            pltpu.VMEM((2, UNROLL + 1, SEG, D), BF16),
            pltpu.VMEM((NSEG, TP, D), BF16),
            pltpu.VMEM((NSEG * TP, D), BF16),
            pltpu.VMEM((NP, NSEG * TP, 2 * PW), F32),
            pltpu.VMEM((NSEG, SEG, D), BF16),
            pltpu.VMEM((M + SEG, D), F32),
            pltpu.VMEM((SEG, D), F32),
            pltpu.SemaphoreType.DMA((NP * 3,)),
            pltpu.SemaphoreType.DMA((NP,)),
            pltpu.SemaphoreType.DMA((4,)),
            pltpu.SemaphoreType.DMA((2,)),
            pltpu.SemaphoreType.DMA((1,)),
        ],
        compiler_params=pltpu.CompilerParams(vmem_limit_bytes=120 * 1024 * 1024,
                                             disable_bounds_checks=True),
    )(A_x.reshape(NSEG, SEG, D), A_mem0.reshape(M, D), heads_major(A_Wq), heads_major(A_Wk),
      heads_major(A_Wv), A_Wo.reshape(H * DH, D), B_w_gate, B_w_up, B_w_down)
    return out.reshape(B, S, D)
```
